```python
import jax
import jax.numpy as jnp

def _softmax(x, axis=-1):
    return jax.nn.softmax(x, axis=axis)

def _gelu(x):
    return jax.nn.gelu(x, approximate=True)

def _silu(x):
    return jax.nn.silu(x)

def _sigmoid(x):
    return jax.nn.sigmoid(x)

def _layernorm(x, axis=-1, eps=1e-05):
    m = jnp.mean(x, axis=axis, keepdims=True)
    v = jnp.var(x, axis=axis, keepdims=True)
    return (x - m) / jnp.sqrt(v + eps)

def _scatter_add(tgt, idx, src, axis=0):
    return tgt.at[idx].add(src)

def _segment_sum(src, seg, n):
    return jax.ops.segment_sum(src, seg, n)

class _Rng:

    def __init__(self, key):
        self._k = key

    def _next(self):
        self._k, sub = jax.random.split(self._k)
        return sub

    def normal(self, shape):
        return jax.random.normal(self._next(), shape, dtype=jnp.bfloat16)

    def randint(self, lo, hi, shape):
        return jax.random.randint(self._next(), shape, lo, hi, dtype=jnp.int32)

    def uniform(self, shape, lo=0.0, hi=1.0):
        return jax.random.uniform(self._next(), shape, jnp.bfloat16, lo, hi)

    def permutation(self, n):
        return jax.random.permutation(self._next(), n)
kernel_name = 'standalone__dilated_atrous__vision'

def setup_inputs():
    _rng = _Rng(jax.random.key(int.from_bytes(__import__("os").urandom(4), "little")))
    _w = lambda a: (lambda t: t.astype(jnp.bfloat16) if jnp.issubdtype(t.dtype, jnp.floating) else t)(jnp.asarray(a))
    H = W = 384
    C = 384
    k = 1
    return {'x': _w((lambda *s: _rng.normal(s) * 0.05)(1, H, W, C)), 'w': _w((lambda *s: _rng.normal(s) * 0.05)(k, k, C, C) * (1.0 / (k * C ** 0.5)))}

def reference(x, w):
    B, H, W, C = x.shape
    k = 1
    rate = 2
    pad = (k - 1) * rate // 2
    xp = jnp.pad(x, ((0, 0), (pad, pad), (pad, pad), (0, 0)))
    out = jnp.zeros_like(x)
    for i in range(k):
        for j in range(k):
            tap = xp[:, i * rate:i * rate + H, j * rate:j * rate + W, :].copy()
            out = out + jnp.einsum('bhwc,co->bhwo', tap, w[i, j])
    return out
```

```python
import jax
import jax.numpy as jnp
from jax import lax
import jax.experimental.pallas as pl
import jax.experimental.pallas.tpu as pltpu

_UNIT = 128
_PIECE = 128
_STREAMS = 12
_SLAB_UNITS = 16
_STEP_UNITS = 6
_LEAD = 3
_RING = 8
_W_SLABS = 6
_W_SLAB_ROWS = 4096
_W_ROWS = 64
_W_FIRST = 12
_W_PER_STEP = 11


def _split(i, n):
    assert n & (n - 1) == 0
    return lax.shift_right_logical(i, n.bit_length() - 1), i & (n - 1)


def _from_tiles(t):
    r = t.shape[0] // 3
    u = pltpu.bitcast(t, jnp.int32).reshape(r // 16, 3, 8, 128)
    v0, v1, v2 = u[:, 0], u[:, 1], u[:, 2]
    first = lax.broadcasted_iota(jnp.int32, v0.shape, 1) < 4
    blocks = (jnp.where(first, v0, v1),
              pltpu.roll(jnp.where(first, v2, v0), 4, 1),
              jnp.where(first, v1, v2))
    return jnp.concatenate(
        [pltpu.bitcast(b.reshape(r // 2, 128), t.dtype) for b in blocks], axis=1)


def _to_tiles(m):
    r = m.shape[0]
    blocks = [m[:, n * 128:(n + 1) * 128].reshape(r // 8, 8, 128) for n in range(3)]
    return jnp.stack(blocks, axis=1).reshape(3 * r, 128)


@jax.jit
def pallas_standalone__dilated_atrous__vision_kernel(
    x: jax.Array,
    w: jax.Array,
):
    B, H, W, C = x.shape
    assert w.shape == (1, 1, C, C) and C == 3 * 128
    assert x.dtype == w.dtype == jnp.bfloat16
    M = B * H * W
    unit_rows = 3 * _UNIT
    n_units = M // _UNIT
    n_steps = n_units // _STEP_UNITS

    group_units = _STREAMS * _SLAB_UNITS
    n_rounds = n_units // _STREAMS
    round_reads = _STREAMS * unit_rows // _PIECE
    round_steps = _STREAMS // _STEP_UNITS
    assert n_units * _UNIT == M and n_units % group_units == 0
    assert round_steps * _STEP_UNITS == _STREAMS and round_steps >= 2 and _LEAD < _RING

    n_slabs = 3 * M // _W_SLAB_ROWS
    group_writes = _W_SLAB_ROWS // _W_ROWS
    n_writes = n_slabs // _W_SLABS * group_writes
    assert n_slabs * _W_SLAB_ROWS == 3 * M and n_slabs % _W_SLABS == 0

    def kernel_function(x_hbm, w_hbm, o_hbm, buf, wbuf):
        slabs = buf.reshape(n_slabs, _W_SLAB_ROWS, 128)

        def run(read_sems, w_sem, out_sem):
            def round_starts(t):
                g, j = _split(t, _SLAB_UNITS)
                base = (g * group_units + j) * unit_rows
                sem = read_sems.at[t & (_RING - 1)]

                def start(k):
                    r, s = divmod(k, _STREAMS)
                    row = base + s * _SLAB_UNITS * unit_rows + r * _PIECE
                    rows = pl.ds(pl.multiple_of(row, _PIECE), _PIECE)
                    pltpu.make_async_copy(
                        x_hbm.at[rows], buf.at[rows], sem).start(priority=s % 2)

                return [lambda k=k: start(k) for k in range(round_reads)]

            def wait_round(t):
                rows = pl.ds(0, round_reads * _PIECE)
                pltpu.make_async_copy(
                    x_hbm.at[rows], buf.at[rows], read_sems.at[t & (_RING - 1)]).wait()

            def start_writes(lo, hi):
                def start(k, _):
                    g, j = _split(k, group_writes)
                    idx = (pl.ds(g * _W_SLABS, _W_SLABS),
                           pl.ds(pl.multiple_of(j * _W_ROWS, _W_ROWS), _W_ROWS))
                    pltpu.make_async_copy(slabs.at[idx], o_hbm.at[idx], out_sem).start()

                lax.fori_loop(lo, hi, start, None)

            def matmul_step(c, starts=()):
                in_first = c < group_units // _STEP_UNITS
                j = lax.div(c, round_steps)
                part = c - j * round_steps
                unit = jnp.where(
                    in_first, part * _STEP_UNITS * _SLAB_UNITS + j, c * _STEP_UNITS)
                hop = jnp.where(in_first, _SLAB_UNITS, 1)
                rows = [pl.multiple_of((unit + k * hop) * unit_rows, unit_rows)
                        for k in range(_STEP_UNITS)]
                parts = max(len(starts) // _STEP_UNITS, 1)
                assert len(starts) in (0, parts * _STEP_UNITS)
                cuts = [p * (unit_rows // 16) // parts * 16 for p in range(parts + 1)]
                tiles = buf[pl.ds(rows[0], unit_rows), :]
                for k in range(_STEP_UNITS):
                    lhs = _from_tiles(tiles)
                    if k + 1 < _STEP_UNITS:
                        tiles = buf[pl.ds(rows[k + 1], unit_rows), :]
                    res = jnp.dot(lhs, wbuf[...], preferred_element_type=jnp.float32)
                    res = _to_tiles(res).astype(buf.dtype)
                    for p, (lo, hi) in enumerate(zip(cuts, cuts[1:])):
                        if starts:
                            starts[k * parts + p]()
                        buf[pl.ds(rows[k] + lo, hi - lo), :] = res[lo:hi]

            w_copy = pltpu.make_async_copy(w_hbm, wbuf, w_sem)
            w_copy.start()

            def lead_round(t, _):
                for start in round_starts(t):
                    start()

            lax.fori_loop(0, _LEAD, lead_round, None)
            w_copy.wait()

            def read_step(c, _):
                wait_round(c)
                matmul_step(c, round_starts(c + _LEAD))

            done = n_rounds - _LEAD
            lax.fori_loop(0, done, read_step, None)
            for t in range(done, n_rounds):
                wait_round(t)

            start_writes(0, _W_FIRST)

            def write_step(c, started):
                ready = lax.div(c * _STEP_UNITS * unit_rows, _W_SLABS * _W_SLAB_ROWS)
                target = jnp.minimum(
                    ready * group_writes, _W_FIRST + (c - done + 1) * _W_PER_STEP)
                start_writes(started, target)
                matmul_step(c)
                return target

            started = lax.fori_loop(done, n_steps, write_step, jnp.int32(_W_FIRST))
            start_writes(started, n_writes)
            pltpu.make_async_copy(slabs, o_hbm, out_sem).wait()

        pl.run_scoped(
            run,
            pltpu.SemaphoreType.DMA((_RING,)),
            pltpu.SemaphoreType.DMA(()),
            pltpu.SemaphoreType.DMA(()),
        )

    x_tiles = x.reshape(M // 8, 8, 3, 128).transpose(0, 2, 1, 3).reshape(3 * M, 128)
    out = pl.pallas_call(
        kernel_function,
        in_specs=[
            pl.BlockSpec(memory_space=pl.ANY),
            pl.BlockSpec(memory_space=pl.ANY),
        ],
        out_specs=pl.BlockSpec(memory_space=pl.ANY),
        out_shape=jax.ShapeDtypeStruct((n_slabs, _W_SLAB_ROWS, 128), x.dtype),
        scratch_shapes=[
            pltpu.VMEM((3 * M, 128), x.dtype),
            pltpu.VMEM((C, C), w.dtype),
        ],
        compiler_params=pltpu.CompilerParams(
            vmem_limit_bytes=120 * 2**20, disable_bounds_checks=True),
    )(x_tiles, w.reshape(C, C))
    return out.reshape(M // 8, 3, 8, 128).transpose(0, 2, 1, 3).reshape(B, H, W, C)
```

```python
import jax
import jax.numpy as jnp
from jax import lax
import jax.experimental.pallas as pl
import jax.experimental.pallas.tpu as pltpu

_SLAB = 4096
_UNIT = 384
_STEP_UNITS = 9

_READ = 128
_STREAMS = 54
_LEAD = 4
_RING = 8
_TAIL = 12

_WRITE = 64
_WRITE_SLABS = 6
_FIRST_WRITES = 24
_STEP_WRITES = 15


def _split(i, n):
    assert n & (n - 1) == 0
    return i >> (n.bit_length() - 1), i & (n - 1)


def _from_tiles(t):
    r = t.shape[0] // 3
    u = pltpu.bitcast(t, jnp.int32).reshape(r // 16, 3, 8, 128)
    v0, v1, v2 = u[:, 0], u[:, 1], u[:, 2]
    first = lax.broadcasted_iota(jnp.int32, v0.shape, 1) < 4
    blocks = (jnp.where(first, v0, v1),
              pltpu.roll(jnp.where(first, v2, v0), 4, 1),
              jnp.where(first, v1, v2))
    return jnp.concatenate(
        [pltpu.bitcast(b.reshape(r // 2, 128), t.dtype) for b in blocks], axis=1)


def _to_tiles(m):
    r = m.shape[0]
    blocks = [m[:, n * 128:(n + 1) * 128].reshape(r // 8, 8, 128) for n in range(3)]
    return jnp.stack(blocks, axis=1).reshape(3 * r, 128)


@jax.jit
def pallas_standalone__dilated_atrous__vision_kernel(
    x: jax.Array,
    w: jax.Array,
):
    B, H, W, C = x.shape
    assert w.shape == (1, 1, C, C) and C == 3 * 128
    assert x.dtype == w.dtype == jnp.bfloat16
    M = B * H * W
    n_slabs = 3 * M // _SLAB
    n_steps = 3 * M // (_STEP_UNITS * _UNIT)
    assert n_slabs * _SLAB == n_steps * _STEP_UNITS * _UNIT == 3 * M

    group_rounds = _SLAB // _READ
    n_rounds = n_slabs // _STREAMS * group_rounds
    queue_reads = _STREAMS // 2
    read_steps = n_rounds - _LEAD
    assert n_slabs % _STREAMS == 0 and _TAIL <= queue_reads and _LEAD + 2 <= _RING
    assert _UNIT == 3 * _READ and group_rounds == 32
    assert read_steps * _STEP_UNITS * _UNIT <= _STREAMS * _SLAB
    assert read_steps >= group_rounds

    group_writes = _SLAB // _WRITE
    n_writes = n_slabs // _WRITE_SLABS * group_writes
    assert n_slabs % _WRITE_SLABS == 0
    for c in range(read_steps, n_steps):
        finished = c * _STEP_UNITS * _UNIT // (_WRITE_SLABS * _SLAB) * group_writes
        assert _FIRST_WRITES + (c - read_steps + 1) * _STEP_WRITES <= finished

    def kernel_function(x_hbm, w_hbm, o_hbm, buf, wbuf):
        slabs = buf.reshape(n_slabs, _SLAB, 128)

        def matmul_step(c, starts):
            early = c < group_rounds
            unit = jnp.where(early, (11 * c) & (group_rounds - 1), _STEP_UNITS * c)
            hop = jnp.where(early, group_rounds, 1)
            rows = [pl.multiple_of((unit + k * hop) * _UNIT, _READ)
                    for k in range(_STEP_UNITS)]
            edges = [k * len(starts) // _STEP_UNITS for k in range(_STEP_UNITS + 1)]
            tiles = buf[pl.ds(rows[0], _UNIT), :]
            for k in range(_STEP_UNITS):
                lhs = _from_tiles(tiles)
                if k + 1 < _STEP_UNITS:
                    tiles = buf[pl.ds(rows[k + 1], _UNIT), :]
                res = jnp.dot(lhs, wbuf[...], preferred_element_type=jnp.float32)
                res = _to_tiles(res).astype(buf.dtype)
                mine = starts[edges[k]:edges[k + 1]]
                cuts = [p * (_UNIT // 16) // len(mine) * 16 for p in range(len(mine) + 1)]
                for start, lo, hi in zip(mine, cuts, cuts[1:]):
                    start()
                    buf[pl.ds(rows[k] + lo, hi - lo), :] = res[lo:hi]

        def run(round_sems, tail_sem, w_sem, out_sem):
            def start_read(r, k, queue, sem=None):
                g, j = _split(r, group_rounds)
                row = (g * _STREAMS + 2 * k + queue) * _SLAB + j * _READ
                rows = pl.ds(pl.multiple_of(row, _READ), _READ)
                sem = round_sems.at[r & (_RING - 1)] if sem is None else sem
                pltpu.make_async_copy(x_hbm.at[rows], buf.at[rows], sem).start(priority=queue)

            def step_reads(r):
                return [lambda k=k, queue=queue: start_read(r + queue, k, queue)
                        for k in range(queue_reads) for queue in range(2)]

            def wait_reads(r, lo=0, hi=_STREAMS, sem=None):
                g, j = _split(r, group_rounds)
                done = slabs.at[pl.ds(g * _STREAMS + lo, hi - lo),
                                pl.ds(pl.multiple_of(j * _READ, _READ), _READ)]
                sem = round_sems.at[r & (_RING - 1)] if sem is None else sem
                pltpu.make_async_copy(done, done, sem).wait()

            def start_write(k):
                g, j = _split(k, group_writes)
                idx = (pl.ds(g * _WRITE_SLABS, _WRITE_SLABS),
                       pl.ds(pl.multiple_of(j * _WRITE, _WRITE), _WRITE))
                pltpu.make_async_copy(slabs.at[idx], o_hbm.at[idx], out_sem).start()

            for k in range(queue_reads):
                start_read(jnp.int32(0), k, 1)
            w_copy = pltpu.make_async_copy(w_hbm, wbuf, w_sem)
            w_copy.start()

            def lead_round(r, _):
                for start in step_reads(r):
                    start()

            lax.fori_loop(0, _LEAD, lead_round, None)
            w_copy.wait()
            wait_reads(jnp.int32(0))
            wait_reads(jnp.int32(1))

            def read_step(c, _):
                wait_reads(c + 2)
                matmul_step(c, step_reads(c + _LEAD))

            lax.fori_loop(0, read_steps - 2, read_step, None)

            last = jnp.int32(n_rounds - 1)
            starts = step_reads(last - 1)
            for k in range(queue_reads - _TAIL, queue_reads):
                starts[2 * k + 1] = lambda k=k: start_read(last, k, 1, tail_sem)
            wait_reads(last - _LEAD + 1)
            matmul_step(last - _LEAD - 1, starts)
            wait_reads(last - _LEAD + 2)
            matmul_step(last - _LEAD, step_reads(last)[::2])
            for back in range(_LEAD - 3, 0, -1):
                wait_reads(last - back)
            wait_reads(last, hi=_STREAMS - _TAIL)

            lax.fori_loop(0, _FIRST_WRITES, lambda k, _: start_write(k), None)
            wait_reads(last, lo=_STREAMS - _TAIL, sem=tail_sem)

            def write_step(c, _):
                k0 = _FIRST_WRITES + (c - read_steps) * _STEP_WRITES
                matmul_step(
                    c, [lambda i=i: start_write(k0 + i) for i in range(_STEP_WRITES)])

            lax.fori_loop(read_steps, n_steps, write_step, None)
            lax.fori_loop(_FIRST_WRITES + (n_steps - read_steps) * _STEP_WRITES, n_writes,
                          lambda k, _: start_write(k), None)
            pltpu.make_async_copy(slabs, o_hbm, out_sem).wait()

        pl.run_scoped(
            run,
            pltpu.SemaphoreType.DMA((_RING,)),
            pltpu.SemaphoreType.DMA(()),
            pltpu.SemaphoreType.DMA(()),
            pltpu.SemaphoreType.DMA(()),
        )

    x_tiles = x.reshape(M // 8, 8, 3, 128).transpose(0, 2, 1, 3).reshape(3 * M, 128)
    out = pl.pallas_call(
        kernel_function,
        in_specs=[
            pl.BlockSpec(memory_space=pl.ANY),
            pl.BlockSpec(memory_space=pl.ANY),
        ],
        out_specs=pl.BlockSpec(memory_space=pl.ANY),
        out_shape=jax.ShapeDtypeStruct((n_slabs, _SLAB, 128), x.dtype),
        scratch_shapes=[
            pltpu.VMEM((3 * M, 128), x.dtype),
            pltpu.VMEM((C, C), w.dtype),
        ],
        compiler_params=pltpu.CompilerParams(
            vmem_limit_bytes=120 * 2**20, disable_bounds_checks=True),
    )(x_tiles, w.reshape(C, C))
    return out.reshape(M // 8, 3, 8, 128).transpose(0, 2, 1, 3).reshape(B, H, W, C)
```

```python
import jax
import jax.numpy as jnp
from jax import lax
import jax.experimental.pallas as pl
import jax.experimental.pallas.tpu as pltpu

_SLAB = 4096
_UNIT = 384
_STEP_UNITS = 9

_READ = 128
_STREAMS = 54
_LEAD = 4
_RING = 8
_TAIL = 24

_WRITE = 64
_WRITE_SLABS = 6
_FIRST_WRITES = 24
_STEP_WRITES = 15


def _split(i, n):
    assert n & (n - 1) == 0
    return i >> (n.bit_length() - 1), i & (n - 1)


def _from_tiles(t):
    r = t.shape[0] // 3
    u = pltpu.bitcast(t, jnp.int32).reshape(r // 16, 3, 8, 128)
    v0, v1, v2 = u[:, 0], u[:, 1], u[:, 2]
    first = lax.broadcasted_iota(jnp.int32, v0.shape, 1) < 4
    blocks = (jnp.where(first, v0, v1),
              pltpu.roll(jnp.where(first, v2, v0), 4, 1),
              jnp.where(first, v1, v2))
    return jnp.concatenate(
        [pltpu.bitcast(b.reshape(r // 2, 128), t.dtype) for b in blocks], axis=1)


def _to_tiles(m):
    r = m.shape[0]
    blocks = [m[:, n * 128:(n + 1) * 128].reshape(r // 8, 8, 128) for n in range(3)]
    return jnp.stack(blocks, axis=1).reshape(3 * r, 128)


@jax.jit
def pallas_standalone__dilated_atrous__vision_kernel(
    x: jax.Array,
    w: jax.Array,
):
    B, H, W, C = x.shape
    assert w.shape == (1, 1, C, C) and C == 3 * 128
    assert x.dtype == w.dtype == jnp.bfloat16
    M = B * H * W
    n_slabs = 3 * M // _SLAB
    n_steps = 3 * M // (_STEP_UNITS * _UNIT)
    assert n_slabs * _SLAB == n_steps * _STEP_UNITS * _UNIT == 3 * M

    group_rounds = _SLAB // _READ
    n_rounds = n_slabs // _STREAMS * group_rounds
    read_steps = n_rounds - _LEAD
    assert n_slabs % _STREAMS == 0 and _TAIL < _STREAMS and _LEAD + 2 <= _RING
    assert _UNIT == 3 * _READ and group_rounds == 32
    assert read_steps * _STEP_UNITS * _UNIT <= _STREAMS * _SLAB
    assert read_steps >= group_rounds

    group_writes = _SLAB // _WRITE
    n_writes = n_slabs // _WRITE_SLABS * group_writes
    assert n_slabs % _WRITE_SLABS == 0
    for c in range(read_steps, n_steps):
        finished = c * _STEP_UNITS * _UNIT // (_WRITE_SLABS * _SLAB) * group_writes
        assert _FIRST_WRITES + (c - read_steps + 1) * _STEP_WRITES <= finished

    def kernel_function(x_hbm, w_hbm, o_hbm, buf, wbuf):
        slabs = buf.reshape(n_slabs, _SLAB, 128)

        def matmul_step(c, starts):
            early = c < group_rounds
            unit = jnp.where(early, (11 * c) & (group_rounds - 1), _STEP_UNITS * c)
            hop = jnp.where(early, group_rounds, 1)
            rows = [pl.multiple_of((unit + k * hop) * _UNIT, _READ)
                    for k in range(_STEP_UNITS)]
            edges = [k * len(starts) // _STEP_UNITS for k in range(_STEP_UNITS + 1)]
            tiles = buf[pl.ds(rows[0], _UNIT), :]
            for k in range(_STEP_UNITS):
                lhs = _from_tiles(tiles)
                if k + 1 < _STEP_UNITS:
                    tiles = buf[pl.ds(rows[k + 1], _UNIT), :]
                res = jnp.dot(lhs, wbuf[...], preferred_element_type=jnp.float32)
                res = _to_tiles(res).astype(buf.dtype)
                mine = starts[edges[k]:edges[k + 1]]
                cuts = [p * (_UNIT // 16) // len(mine) * 16 for p in range(len(mine) + 1)]
                for start, lo, hi in zip(mine, cuts, cuts[1:]):
                    start()
                    buf[pl.ds(rows[k] + lo, hi - lo), :] = res[lo:hi]

        def run(round_sems, tail_sem, w_sem, out_sem):
            def start_read(r, s, is_last=False):
                g, j = _split(r, group_rounds)
                row = (g * _STREAMS + s) * _SLAB + j * _READ
                rows = pl.ds(pl.multiple_of(row, _READ), _READ)
                in_tail = is_last and s >= _STREAMS - _TAIL
                sem = tail_sem if in_tail else round_sems.at[r & (_RING - 1)]
                pltpu.make_async_copy(x_hbm.at[rows], buf.at[rows], sem).start(priority=s % 2)

            def step_reads(r, last_queue=None):
                return [lambda s=s: start_read(r + s % 2, s, s % 2 == last_queue)
                        for s in range(_STREAMS)]

            def wait_reads(r, lo=0, hi=_STREAMS, sem=None):
                g, j = _split(r, group_rounds)
                done = slabs.at[pl.ds(g * _STREAMS + lo, hi - lo),
                                pl.ds(pl.multiple_of(j * _READ, _READ), _READ)]
                sem = round_sems.at[r & (_RING - 1)] if sem is None else sem
                pltpu.make_async_copy(done, done, sem).wait()

            def start_write(k):
                g, j = _split(k, group_writes)
                idx = (pl.ds(g * _WRITE_SLABS, _WRITE_SLABS),
                       pl.ds(pl.multiple_of(j * _WRITE, _WRITE), _WRITE))
                pltpu.make_async_copy(slabs.at[idx], o_hbm.at[idx], out_sem).start()

            for s in range(1, _STREAMS, 2):
                start_read(jnp.int32(0), s)
            w_copy = pltpu.make_async_copy(w_hbm, wbuf, w_sem)
            w_copy.start()

            def lead_round(r, _):
                for start in step_reads(r):
                    start()

            lax.fori_loop(0, _LEAD, lead_round, None)
            w_copy.wait()
            wait_reads(jnp.int32(0))
            wait_reads(jnp.int32(1))

            def read_step(c, _):
                wait_reads(c + 2)
                matmul_step(c, step_reads(c + _LEAD))

            lax.fori_loop(0, read_steps - 2, read_step, None)

            last = jnp.int32(n_rounds - 1)
            wait_reads(last - _LEAD + 1)
            matmul_step(last - _LEAD - 1, step_reads(last - 1, last_queue=1))
            wait_reads(last - _LEAD + 2)
            matmul_step(last - _LEAD, step_reads(last, last_queue=0)[::2])
            for back in range(_LEAD - 3, 0, -1):
                wait_reads(last - back)
            wait_reads(last, hi=_STREAMS - _TAIL)

            lax.fori_loop(0, _FIRST_WRITES, lambda k, _: start_write(k), None)
            wait_reads(last, lo=_STREAMS - _TAIL, sem=tail_sem)

            def write_step(c, _):
                k0 = _FIRST_WRITES + (c - read_steps) * _STEP_WRITES
                matmul_step(
                    c, [lambda i=i: start_write(k0 + i) for i in range(_STEP_WRITES)])

            lax.fori_loop(read_steps, n_steps, write_step, None)
            lax.fori_loop(_FIRST_WRITES + (n_steps - read_steps) * _STEP_WRITES, n_writes,
                          lambda k, _: start_write(k), None)
            pltpu.make_async_copy(slabs, o_hbm, out_sem).wait()

        pl.run_scoped(
            run,
            pltpu.SemaphoreType.DMA((_RING,)),
            pltpu.SemaphoreType.DMA(()),
            pltpu.SemaphoreType.DMA(()),
            pltpu.SemaphoreType.DMA(()),
        )

    x_tiles = x.reshape(M // 8, 8, 3, 128).transpose(0, 2, 1, 3).reshape(3 * M, 128)
    out = pl.pallas_call(
        kernel_function,
        in_specs=[
            pl.BlockSpec(memory_space=pl.ANY),
            pl.BlockSpec(memory_space=pl.ANY),
        ],
        out_specs=pl.BlockSpec(memory_space=pl.ANY),
        out_shape=jax.ShapeDtypeStruct((n_slabs, _SLAB, 128), x.dtype),
        scratch_shapes=[
            pltpu.VMEM((3 * M, 128), x.dtype),
            pltpu.VMEM((C, C), w.dtype),
        ],
        compiler_params=pltpu.CompilerParams(
            vmem_limit_bytes=120 * 2**20, disable_bounds_checks=True),
    )(x_tiles, w.reshape(C, C))
    return out.reshape(M // 8, 3, 8, 128).transpose(0, 2, 1, 3).reshape(B, H, W, C)
```

```python
import jax
import jax.numpy as jnp
from jax import lax
import jax.experimental.pallas as pl
import jax.experimental.pallas.tpu as pltpu

_SLAB = 4096
_PIECE = 128
_STEP_DOTS = 9
_STORE = 64

_STREAMS = 54
_LEAD = 4
_RING = 8
_TAIL = 24

_WRITE = 64
_WRITE_SLABS = 6
_FIRST_WRITES = 24
_STEP_WRITES = 15


def _split(i, n):
    assert n & (n - 1) == 0
    return i >> (n.bit_length() - 1), i & (n - 1)


def _from_tiles(t):
    r = t.shape[0] // 3
    u = pltpu.bitcast(t, jnp.int32).reshape(r // 16, 3, 8, 128)
    v0, v1, v2 = u[:, 0], u[:, 1], u[:, 2]
    first = lax.broadcasted_iota(jnp.int32, v0.shape, 1) < 4
    blocks = (jnp.where(first, v0, v1),
              pltpu.roll(jnp.where(first, v2, v0), 4, 1),
              jnp.where(first, v1, v2))
    return jnp.concatenate(
        [pltpu.bitcast(b.reshape(r // 2, 128), t.dtype) for b in blocks], axis=1)


def _to_tiles(m):
    r = m.shape[0]
    blocks = [m[:, n * 128:(n + 1) * 128].reshape(r // 8, 8, 128) for n in range(3)]
    return jnp.stack(blocks, axis=1).reshape(3 * r, 128)


@jax.jit
def pallas_standalone__dilated_atrous__vision_kernel(
    x: jax.Array,
    w: jax.Array,
):
    B, H, W, C = x.shape
    assert w.shape == (1, 1, C, C) and C == 3 * 128
    assert x.dtype == w.dtype == jnp.bfloat16
    M = B * H * W
    step_rows = _STEP_DOTS * 3 * _PIECE
    n_slabs = 3 * M // _SLAB
    n_steps = 3 * M // step_rows
    assert n_slabs * _SLAB == n_steps * step_rows == 3 * M

    slab_pieces = _SLAB // _PIECE
    n_rounds = n_slabs // _STREAMS * slab_pieces
    read_steps = n_rounds - _LEAD
    assert n_slabs % _STREAMS == 0 and _TAIL < _STREAMS and _LEAD + 2 <= _RING
    assert read_steps * step_rows <= _STREAMS * _SLAB
    assert slab_pieces == 32 and read_steps >= slab_pieces

    group_writes = _SLAB // _WRITE
    n_writes = n_slabs // _WRITE_SLABS * group_writes
    assert n_slabs % _WRITE_SLABS == 0
    for c in range(read_steps, n_steps):
        finished = c * step_rows // (_WRITE_SLABS * _SLAB) * group_writes
        assert _FIRST_WRITES + (c - read_steps + 1) * _STEP_WRITES <= finished

    def kernel_function(x_hbm, w_hbm, o_hbm, buf, wbuf):
        def matmul_step(c, starts):
            early = c < slab_pieces
            first = jnp.where(early, (11 * c) & (slab_pieces - 1), _STEP_DOTS * c)
            hop = jnp.where(early, slab_pieces, 1)

            def rows(k, lo, n):
                s, j = _split(3 * (first + k * hop) + lo // _PIECE, slab_pieces)
                return s, pl.ds(pl.multiple_of(j * _PIECE + lo % _PIECE, n), n)

            def load(k):
                return jnp.concatenate(
                    [buf[rows(k, i * _PIECE, _PIECE)] for i in range(3)], axis=0)

            stores = step_rows // _STORE
            before = {i * stores // len(starts): start for i, start in enumerate(starts)}
            assert len(before) == len(starts)
            tiles = load(0)
            for k in range(_STEP_DOTS):
                lhs = _from_tiles(tiles)
                if k + 1 < _STEP_DOTS:
                    tiles = load(k + 1)
                res = jnp.dot(lhs, wbuf[...], preferred_element_type=jnp.float32)
                res = _to_tiles(res).astype(buf.dtype)
                for lo in range(0, 3 * _PIECE, _STORE):
                    store = (k * 3 * _PIECE + lo) // _STORE
                    if store in before:
                        before[store]()
                    buf[rows(k, lo, _STORE)] = res[lo:lo + _STORE]

        def run(round_sems, tail_sem, w_sem, out_sem):
            def start_read(r, s, is_last=False):
                g, j = _split(r, slab_pieces)
                idx = (g * _STREAMS + s, pl.ds(pl.multiple_of(j * _PIECE, _PIECE), _PIECE))
                in_tail = is_last and s >= _STREAMS - _TAIL
                sem = tail_sem if in_tail else round_sems.at[r & (_RING - 1)]
                pltpu.make_async_copy(x_hbm.at[idx], buf.at[idx], sem).start(priority=s % 2)

            def step_reads(r, last_queue=None):
                return [lambda s=s: start_read(r + s % 2, s, s % 2 == last_queue)
                        for s in range(_STREAMS)]

            def wait_reads(r, lo=0, hi=_STREAMS, sem=None):
                g, j = _split(r, slab_pieces)
                done = buf.at[pl.ds(g * _STREAMS + lo, hi - lo),
                              pl.ds(pl.multiple_of(j * _PIECE, _PIECE), _PIECE)]
                sem = round_sems.at[r & (_RING - 1)] if sem is None else sem
                pltpu.make_async_copy(done, done, sem).wait()

            def start_write(k):
                g, j = _split(k, group_writes)
                idx = (pl.ds(g * _WRITE_SLABS, _WRITE_SLABS),
                       pl.ds(pl.multiple_of(j * _WRITE, _WRITE), _WRITE))
                pltpu.make_async_copy(buf.at[idx], o_hbm.at[idx], out_sem).start()

            for s in range(1, _STREAMS, 2):
                start_read(jnp.int32(0), s)
            w_copy = pltpu.make_async_copy(w_hbm, wbuf, w_sem)
            w_copy.start()

            def lead_round(r, _):
                for start in step_reads(r):
                    start()

            lax.fori_loop(0, _LEAD, lead_round, None)
            w_copy.wait()
            wait_reads(jnp.int32(0))
            wait_reads(jnp.int32(1))

            def read_step(c, _):
                wait_reads(c + 2)
                matmul_step(c, step_reads(c + _LEAD))

            lax.fori_loop(0, read_steps - 2, read_step, None)

            last = jnp.int32(n_rounds - 1)
            wait_reads(last - _LEAD + 1)
            matmul_step(last - _LEAD - 1, step_reads(last - 1, last_queue=1))
            wait_reads(last - _LEAD + 2)
            matmul_step(last - _LEAD, step_reads(last, last_queue=0)[::2])
            for back in range(_LEAD - 3, 0, -1):
                wait_reads(last - back)
            wait_reads(last, hi=_STREAMS - _TAIL)

            lax.fori_loop(0, _FIRST_WRITES, lambda k, _: start_write(k), None)
            wait_reads(last, lo=_STREAMS - _TAIL, sem=tail_sem)

            def write_step(c, _):
                k0 = _FIRST_WRITES + (c - read_steps) * _STEP_WRITES
                matmul_step(
                    c, [lambda i=i: start_write(k0 + i) for i in range(_STEP_WRITES)])

            lax.fori_loop(read_steps, n_steps, write_step, None)
            lax.fori_loop(_FIRST_WRITES + (n_steps - read_steps) * _STEP_WRITES, n_writes,
                          lambda k, _: start_write(k), None)
            pltpu.make_async_copy(buf, o_hbm, out_sem).wait()

        pl.run_scoped(
            run,
            pltpu.SemaphoreType.DMA((_RING,)),
            pltpu.SemaphoreType.DMA(()),
            pltpu.SemaphoreType.DMA(()),
            pltpu.SemaphoreType.DMA(()),
        )

    tiles = (n_slabs, _SLAB, 128)
    out = pl.pallas_call(
        kernel_function,
        in_specs=[
            pl.BlockSpec(memory_space=pl.ANY),
            pl.BlockSpec(memory_space=pl.ANY),
        ],
        out_specs=pl.BlockSpec(memory_space=pl.ANY),
        out_shape=jax.ShapeDtypeStruct(tiles, x.dtype),
        scratch_shapes=[
            pltpu.VMEM(tiles, x.dtype),
            pltpu.VMEM((C, C), w.dtype),
        ],
        compiler_params=pltpu.CompilerParams(
            vmem_limit_bytes=120 * 2**20, disable_bounds_checks=True),
    )(x.reshape(M // 8, 8, 3, 128).transpose(0, 2, 1, 3).reshape(tiles), w.reshape(C, C))
    return out.reshape(M // 8, 3, 8, 128).transpose(0, 2, 1, 3).reshape(B, H, W, C)
```
